```python
import os as _os
_os.environ.setdefault("JAX_PLATFORMS", "cpu")
import jax
import jax.numpy as jnp

def _softmax(x, axis=-1):
    return jax.nn.softmax(x, axis=axis)
def _gelu(x):
    return jax.nn.gelu(x, approximate=True)
def _silu(x):
    return jax.nn.silu(x)
def _sigmoid(x):
    return jax.nn.sigmoid(x)
def _layernorm(x, axis=-1, eps=1e-5):
    m = jnp.mean(x, axis=axis, keepdims=True)
    v = jnp.var(x, axis=axis, keepdims=True)
    return (x - m) / jnp.sqrt(v + eps)
def _scatter_add(tgt, idx, src, axis=0):
    return tgt.at[idx].add(src)
def _segment_sum(src, seg, n):
    return jax.ops.segment_sum(src, seg, n)
class _Rng:
    def __init__(self, key):
        self._k = key
    def _next(self):
        self._k, sub = jax.random.split(self._k)
        return sub
    def normal(self, shape):
        return jax.random.normal(self._next(), shape, dtype=jnp.bfloat16)
    def randint(self, lo, hi, shape):
        return jax.random.randint(self._next(), shape, lo, hi, dtype=jnp.int32)
    def uniform(self, shape, lo=0.0, hi=1.0):
        return jax.random.uniform(self._next(), shape, jnp.bfloat16, lo, hi)
    def permutation(self, n):
        return jax.random.permutation(self._next(), n)


kernel_name = 'standalone__gqa_block_cached__near_ridge'

def setup_inputs():
    _rng = _Rng(jax.random.key(int.from_bytes(__import__("os").urandom(4), "little")))
    _w = (lambda a: (lambda t: t.astype(jnp.bfloat16) if jnp.issubdtype(t.dtype, jnp.floating) else t)(jnp.asarray(a)))
    B, Sq, D = 8, 96, 640
    Hq, Hkv, Sk, Dh = 32, 32, 512, 128
    assert Hq % Hkv == 0, (Hq, Hkv)
    return {
        "x": _w((lambda *s: _rng.normal(s) * 0.2)(B, Sq, D)),
        "k_cache": _w((lambda *s: _rng.normal(s) * 3.2)(B, Hkv, Sk, Dh)),
        "v_cache": _w((lambda *s: _rng.normal(s) * 0.05)(B, Hkv, Sk, Dh)),
        "wq": _w((lambda *s: _rng.normal(s) * 0.2)(D, Hq * Dh) * (D ** -0.5)),
        "wo": _w((lambda *s: _rng.normal(s) * 0.05)(Hq * Dh, D) * ((Hq * Dh) ** -0.5)),
    }

def reference(x, k_cache, v_cache, wq, wo):
    B, Sq, D = x.shape
    Hq, Dh = 32, 128
    Hkv = k_cache.shape[1]
    rep = Hq // Hkv
    q = (lambda x, *d: x.transpose(*d))((x @ wq).reshape(B, Sq, Hq, Dh), 0, 2, 1, 3)
    k = jnp.repeat(k_cache, rep, axis=1)
    v = jnp.repeat(v_cache, rep, axis=1)
    scores = jnp.einsum("bhqd,bhkd->bhqk", q, k) * (Dh ** -0.5)
    p = _softmax(scores, axis=-1)
    o = jnp.einsum("bhqk,bhkd->bhqd", p, v)
    return (lambda x, *d: x.transpose(*d))(o, 0, 2, 1, 3).reshape(B, Sq, Hq * Dh) @ wo
```

```python
import functools, contextlib
import jax
import jax.numpy as jnp
import numpy as np
import jax.experimental.pallas as pl
import jax.experimental.pallas.tpu as pltpu

LOG2E = 1.4426950408889634
NT = (((1,), (1,)), ((), ()))

def parse(s):
    ops = []
    for tok in s.split():
        k, a = tok[0], tok[1:]
        if k == "P": ops.append(("QP", [int(c, 16) for c in a]))
        elif k == "K": ops.append(("QK", int(a, 16)))
        elif k == "V": ops.append(("PV", int(a, 16)))
        elif k == "O": ops.append(("OP", [int(c, 16) for c in a]))
        elif k == "I": ops.append(("ISS",))
        else: raise ValueError(tok)
    return ops

SCHED = {
    8: "P0 P1 I K0 P2 K1 V0 P3 K2 V1 P4 K3 V2 P5 K4 V3 P6 K5 V4 P7 K6 V5 K7 V6 O0123 V7 O456 O7",
    4: "P0 P1 I K0 P2 K1 V0 P3 K2 V1 K3 V2 O01 V3 O2 O3",
    2: "P0 P1 I K0 K1 V0 V1 O0 O1",
}

def make(HG=8, LA=4, R=None, nosc=0, vmem=120 * 2**20, sched=None, unroll=1, scopes=0, nobc=1, flags=None):
    @jax.jit
    def fn(x, k_cache, v_cache, wq, wo):
        B, Sq, D = x.shape
        _, H, Sk, Dh = k_cache.shape
        c = (Dh ** -0.5) * LOG2E
        NG = H // HG
        T = NG * B
        W = HG * Dh
        ops = parse(sched or SCHED[HG])
        RR = R or LA
        assert RR >= LA and LA <= B
        sh = B.bit_length() - 1
        assert 1 << sh == B

        def kernel(x_hbm, k_hbm, v_hbm, wq_hbm, wo_hbm, out_hbm,
                   xb, kb, vb, wqb, wob, acc, outb, kvsem, wsem):
            sc = (lambda n: jax.named_scope(n)) if scopes else (lambda n: contextlib.nullcontext())
            def ring(t):
                if RR & (RR - 1) == 0:
                    return jax.lax.bitwise_and(t, RR - 1)
                return jax.lax.rem(t, RR)
            def gb(t):
                return jax.lax.shift_right_logical(t, sh), jax.lax.bitwise_and(t, B - 1)
            def kcp(t, g, b):
                hs = pl.ds(pl.multiple_of(g * HG, HG), HG)
                return pltpu.make_async_copy(k_hbm.at[b, hs], kb.at[b, hs], kvsem.at[ring(t)])
            def vcp(t, g, b):
                hs = pl.ds(pl.multiple_of(g * HG, HG), HG)
                return pltpu.make_async_copy(v_hbm.at[b, hs], vb.at[b, hs], kvsem.at[ring(t)])
            def wqcp(g):
                return pltpu.make_async_copy(wq_hbm.at[:, pl.ds(pl.multiple_of(g * W, W), W)], wqb.at[g], wsem.at[0])
            def wocp(g):
                return pltpu.make_async_copy(wo_hbm.at[pl.ds(pl.multiple_of(g * W, W), W), :], wob.at[g], wsem.at[0])
            ocp0 = pltpu.make_async_copy(outb.at[pl.ds(0, B - 1)], out_hbm.at[pl.ds(0, B - 1)], wsem.at[2])
            ocp1 = pltpu.make_async_copy(outb.at[pl.ds(B - 1, 1)], out_hbm.at[pl.ds(B - 1, 1)], wsem.at[2])
            xcp = pltpu.make_async_copy(x_hbm, xb, wsem.at[1])

            def issue(tn, guard):
                gn, bn = gb(tn)
                if guard:
                    live = tn < T
                    new_g = jnp.logical_and(live, bn == 0)
                else:
                    live = None
                    new_g = bn == 0

                @pl.when(new_g)
                def _():
                    wqcp(gn).start()
                if guard:
                    @pl.when(live)
                    def _():
                        kcp(tn, gn, bn).start()
                    @pl.when(live)
                    def _():
                        vcp(tn, gn, bn).start()
                else:
                    kcp(tn, gn, bn).start()
                    vcp(tn, gn, bn).start()
                @pl.when(new_g)
                def _():
                    wocp(gn).start()

            with sc("p_issue"):
                xcp.start()
                def pro(t, carry):
                    issue(t, False)
                    return carry
                jax.lax.fori_loop(0, min(LA, T), pro, 0)
            with sc("p_zero"):
                acc[...] = jnp.zeros(acc.shape, acc.dtype)
            with sc("p_xw"):
                xcp.wait()

            def body(t, carry):
                g, b = gb(t)
                with sc("wwait"):
                    @pl.when(b == 0)
                    def _():
                        wqcp(g).wait()
                        wocp(g).wait()
                with sc("kwait"):
                    kcp(t, g, b).wait()
                    vcp(t, g, b).wait()

                @pl.when(t == T - 1)
                def _():
                    ocp0.start()

                Q = {}; S = {}; O = {}
                h0 = g * HG
                xv = xb[b]
                a = None
                for op in ops:
                    if op[0] == "QP":
                        js = op[1]
                        j0, n = js[0], len(js)
                        q = jnp.dot(xv, wqb[g, :, j0 * Dh:(j0 + n) * Dh], preferred_element_type=jnp.float32)
                        q = (q * c).astype(jnp.bfloat16)
                        for i, j in enumerate(js):
                            Q[j] = q[:, i * Dh:(i + 1) * Dh] if n > 1 else q
                    elif op[0] == "QK":
                        j = op[1]
                        S[j] = jax.lax.dot_general(Q.pop(j), kb[b, h0 + j], NT, preferred_element_type=jnp.float32)
                    elif op[0] == "ISS":
                        issue(t + LA, True)
                    elif op[0] == "PV":
                        j = op[1]
                        s = S.pop(j)
                        m = jnp.max(s, axis=-1, keepdims=True)
                        p = jnp.exp2(s - m)
                        l = jnp.sum(p, axis=-1, keepdims=True)
                        o = jnp.dot(p.astype(jnp.bfloat16), vb[b, h0 + j], preferred_element_type=jnp.float32)
                        O[j] = (o * pl.reciprocal(l, approx=False)).astype(jnp.bfloat16)
                    elif op[0] == "OP":
                        js = op[1]
                        j0, n = js[0], len(js)
                        ov = jnp.concatenate([O.pop(j) for j in js], axis=1) if n > 1 else O.pop(j0)
                        r = jnp.dot(ov, wob[g, j0 * Dh:(j0 + n) * Dh, :], preferred_element_type=jnp.float32)
                        a = (acc[b] if a is None else a) + r
                acc[b] = a
                outb[b] = a.astype(jnp.bfloat16)
                return carry

            jax.lax.fori_loop(0, T, body, 0, unroll=unroll)
            ocp1.start()
            with sc("owait"):
                ocp0.wait()
                ocp1.wait()

        any_ = pl.BlockSpec(memory_space=pl.ANY)
        return pl.pallas_call(
            kernel,
            in_specs=[any_] * 5,
            out_specs=any_,
            out_shape=jax.ShapeDtypeStruct((B, Sq, D), jnp.bfloat16),
            scratch_shapes=[
                pltpu.VMEM((B, Sq, D), jnp.bfloat16),
                pltpu.VMEM((B, H, Sk, Dh), jnp.bfloat16),
                pltpu.VMEM((B, H, Sk, Dh), jnp.bfloat16),
                pltpu.VMEM((NG, D, W), jnp.bfloat16),
                pltpu.VMEM((NG, W, D), jnp.bfloat16),
                pltpu.VMEM((B, Sq, D), jnp.float32),
                pltpu.VMEM((B, Sq, D), jnp.bfloat16),
                pltpu.SemaphoreType.DMA((RR,)),
                pltpu.SemaphoreType.DMA((3,)),
            ],
            compiler_params=pltpu.CompilerParams(vmem_limit_bytes=vmem, disable_bounds_checks=bool(nobc), disable_semaphore_checks=bool(nosc), flags=flags),
        )(x, k_cache, v_cache, wq, wo)
    return fn


_impl = make(HG=4, LA=3)


@jax.jit
def pallas_standalone__gqa_block_cached__near_ridge_kernel(
    x: jax.Array,
    k_cache: jax.Array,
    v_cache: jax.Array,
    wq: jax.Array,
    wo: jax.Array,
):
    return _impl(x, k_cache, v_cache, wq, wo)
```

```python
import contextlib

import jax
import jax.numpy as jnp
import jax.experimental.pallas as pl
import jax.experimental.pallas.tpu as pltpu

_LOG2E = 1.4426950408889634
_NT = (((1,), (1,)), ((), ()))


def _parse(s):
    return [(tok[0], [int(ch, 16) for ch in tok[1:]]) for tok in s.split()]


_SCHED = {
    4: ("K0 K1 I P0 V0 K2 V1 K3 P1 V2 P2 V3 O01 O2 O3 P3",
        "K0 K1 K2 V0 K3 V1 V2 O0 V3 O1 O2 O3"),
}


def make(HG=4, LA=2, vmem=120 * 2**20, sched=None, sched_last=None, scopes=0, nobc=0, nosc=0, flags=None):
    @jax.jit
    def fn(x, k_cache, v_cache, wq, wo):
        B, Sq, D = x.shape
        _, H, Sk, Dh = k_cache.shape
        NG = H // HG
        T = NG * B
        W = HG * Dh
        c = (Dh ** -0.5) * _LOG2E
        ops_loop = _parse(sched or _SCHED[HG][0])
        ops_last = _parse(sched_last or _SCHED[HG][1])
        shift = B.bit_length() - 1
        assert B == 1 << shift and B > LA >= 2 and LA & (LA - 1) == 0
        assert wq.shape == (D, H * Dh) and v_cache.shape == k_cache.shape

        def kernel(x_hbm, k_hbm, v_hbm, wq_hbm, wo_hbm, out_hbm,
                   xb, kb, vb, wqb, wob, acc, outb, qs, kvsem, wsem):
            sc = (lambda n: jax.named_scope(n)) if scopes else (lambda n: contextlib.nullcontext())

            def gb(t):
                if isinstance(t, int):
                    return t // B, t % B
                return jax.lax.shift_right_logical(t, shift), jax.lax.bitwise_and(t, B - 1)

            def aligned(v, m):
                return v if isinstance(v, int) else pl.multiple_of(v, m)

            def kv_copies(t):
                g, b = gb(t)
                heads = pl.ds(g * HG, HG)
                sem = kvsem.at[t & (LA - 1)]
                return (pltpu.make_async_copy(k_hbm.at[b, heads], kb.at[b, heads], sem),
                        pltpu.make_async_copy(v_hbm.at[b, heads], vb.at[b, heads], sem))

            def w_copies(g):
                cols = pl.ds(aligned(g * W, W), W)
                sem = wsem.at[0]
                return (pltpu.make_async_copy(wq_hbm.at[:, cols], wqb.at[g], sem),
                        pltpu.make_async_copy(wo_hbm.at[cols, :], wob.at[g], sem))

            x_copy = pltpu.make_async_copy(x_hbm, xb, wsem.at[0])

            def out_copy(b0, n):
                rows = pl.ds(b0, n)
                return pltpu.make_async_copy(outb.at[rows], out_hbm.at[rows], wsem.at[0])

            def start(copies):
                for cp in copies:
                    cp.start()

            def wait(copies):
                for cp in copies:
                    cp.wait()

            def enqueue(tn, guard):
                gn, bn = gb(tn)
                next_w = jnp.logical_and(bn == B - 1, gn < NG - 1)
                if guard:
                    @pl.when(next_w)
                    def _():
                        start(w_copies(gn + 1))

                    @pl.when(tn < T)
                    def _():
                        start(kv_copies(tn))
                else:
                    @pl.when(next_w)
                    def _():
                        start(w_copies(gn + 1))

                    start(kv_copies(tn))

            def q_project(g, b, j0, n):
                cols = slice(j0 * Dh, (j0 + n) * Dh)
                q = jnp.dot(xb[b], wqb[g, :, cols], preferred_element_type=jnp.float32)
                qs[:, cols] = (q * c).astype(qs.dtype)

            with sc("p_issue"):
                x_copy.start()
                start(w_copies(0))

                def fill(t, carry):
                    enqueue(t, False)
                    return carry
                jax.lax.fori_loop(0, LA, fill, 0)
            with sc("p_zero"):
                acc[...] = jnp.zeros(acc.shape, acc.dtype)
            with sc("p_xw"):
                x_copy.wait()
                wait(w_copies(0))
            q_project(0, 0, 0, HG)

            def step(t, last):
                g, b = gb(t)
                if last:
                    out_copy(0, B - 1).start()
                else:
                    with sc("wwait"):
                        @pl.when(jnp.logical_and(b == B - 1, g < NG - 1))
                        def _():
                            wait(w_copies(g + 1))
                with sc("kwait"):
                    wait(kv_copies(t))

                h0 = g * HG
                s_of, o_of = {}, {}
                a = None
                for kind, js in (ops_last if last else ops_loop):
                    if kind == "I":
                        enqueue(t + LA, True)
                    elif kind == "P":
                        q_project(*gb(t + 1), js[0], len(js))
                    elif kind == "K":
                        j = js[0]
                        s_of[j] = jax.lax.dot_general(
                            qs[:, j * Dh:(j + 1) * Dh], kb[b, h0 + j], _NT,
                            preferred_element_type=jnp.float32)
                    elif kind == "V":
                        j = js[0]
                        s = s_of.pop(j)
                        m = jnp.max(s, axis=-1, keepdims=True)
                        p = jnp.exp2(s - m)
                        l = jnp.sum(p, axis=-1, keepdims=True)
                        o = jnp.dot(p.astype(vb.dtype), vb[b, h0 + j],
                                    preferred_element_type=jnp.float32)
                        o_of[j] = (o * pl.reciprocal(l, approx=False)).astype(wob.dtype)
                    elif kind == "O":
                        j0, n = js[0], len(js)
                        o = (jnp.concatenate([o_of.pop(j) for j in js], axis=1)
                             if n > 1 else o_of.pop(j0))
                        r = jnp.dot(o, wob[g, j0 * Dh:(j0 + n) * Dh, :],
                                    preferred_element_type=jnp.float32)
                        a = (acc[b] if a is None else a) + r
                if not last:
                    acc[b] = a
                outb[b] = a.astype(outb.dtype)

            def loop_step(t, carry):
                step(t, False)
                return carry
            jax.lax.fori_loop(0, T - 1, loop_step, 0)
            step(T - 1, True)

            out_copy(B - 1, 1).start()
            with sc("owait"):
                out_copy(0, B - 1).wait()
                out_copy(B - 1, 1).wait()

        hbm = pl.BlockSpec(memory_space=pl.ANY)
        return pl.pallas_call(
            kernel,
            in_specs=[hbm] * 5,
            out_specs=hbm,
            out_shape=jax.ShapeDtypeStruct((B, Sq, D), x.dtype),
            scratch_shapes=[
                pltpu.VMEM((B, Sq, D), x.dtype),
                pltpu.VMEM((B, H, Sk, Dh), k_cache.dtype),
                pltpu.VMEM((B, H, Sk, Dh), v_cache.dtype),
                pltpu.VMEM((NG, D, W), wq.dtype),
                pltpu.VMEM((NG, W, D), wo.dtype),
                pltpu.VMEM((B, Sq, D), jnp.float32),
                pltpu.VMEM((B, Sq, D), x.dtype),
                pltpu.VMEM((Sq, W), k_cache.dtype),
                pltpu.SemaphoreType.DMA((LA,)),
                pltpu.SemaphoreType.DMA((1,)),
            ],
            compiler_params=pltpu.CompilerParams(
                vmem_limit_bytes=vmem, disable_bounds_checks=bool(nobc),
                disable_semaphore_checks=bool(nosc), flags=flags),
        )(x, k_cache, v_cache, wq, wo)
    return fn


_impl = make()


@jax.jit
def pallas_standalone__gqa_block_cached__near_ridge_kernel(
    x: jax.Array,
    k_cache: jax.Array,
    v_cache: jax.Array,
    wq: jax.Array,
    wo: jax.Array,
):
    return _impl(x, k_cache, v_cache, wq, wo)
```

```python
import jax
import jax.numpy as jnp
import jax.experimental.pallas as pl
import jax.experimental.pallas.tpu as pltpu

_LOG2E = 1.4426950408889634
_NT = (((1,), (1,)), ((), ()))

_HG = 4
_LA = 2

_STEP = "K0 K1 I K2 V0 K3 V1 O0 V2 O1 V3 O2 P0 O3 P1 P2 P3"
_LAST_STEP = "K0 K1 K2 V0 K3 V1 V2 O0 V3 O1 O2 O3"


def _parse(order):
    return [(tok[0], int(tok[1:]) if tok[1:] else None) for tok in order.split()]


@jax.jit
def pallas_standalone__gqa_block_cached__near_ridge_kernel(
    x: jax.Array,
    k_cache: jax.Array,
    v_cache: jax.Array,
    wq: jax.Array,
    wo: jax.Array,
):
    B, Sq, D = x.shape
    _, H, Sk, Dh = k_cache.shape
    HG, LA = _HG, _LA
    NG = H // HG
    T = NG * B
    W = HG * Dh
    assert wq.shape == (D, H * Dh) and wo.shape == (H * Dh, D)
    assert v_cache.shape == k_cache.shape == (B, H, Sk, Dh) and H % HG == 0
    shift = B.bit_length() - 1
    assert B == 1 << shift and B > LA and LA & (LA - 1) == 0
    q_scale = (Dh ** -0.5) * _LOG2E

    def kernel(x_hbm, k_hbm, v_hbm, wq_hbm, wo_hbm, out_hbm,
               xb, kb, vb, wqb, wob, acc, outb, qs, kvsem, wsem):

        def group_batch(t):
            if isinstance(t, int):
                return t // B, t % B
            return jax.lax.shift_right_logical(t, shift), jax.lax.bitwise_and(t, B - 1)

        def kv_copies(t):
            g, b = group_batch(t)
            heads = pl.ds(g * HG, HG)
            sem = kvsem.at[t & (LA - 1)]
            return (pltpu.make_async_copy(k_hbm.at[b, heads], kb.at[b, heads], sem),
                    pltpu.make_async_copy(v_hbm.at[b, heads], vb.at[b, heads], sem))

        def w_copies(g):
            c0 = g * W if isinstance(g, int) else pl.multiple_of(g * W, W)
            cols = pl.ds(c0, W)
            return (pltpu.make_async_copy(wq_hbm.at[:, cols], wqb.at[g], wsem.at[0]),
                    pltpu.make_async_copy(wo_hbm.at[cols, :], wob.at[g], wsem.at[0]))

        def x_copies():
            return (pltpu.make_async_copy(x_hbm, xb, wsem.at[0]),)

        def out_copies(b0, n):
            rows = pl.ds(b0, n)
            return (pltpu.make_async_copy(outb.at[rows], out_hbm.at[rows], wsem.at[0]),)

        def start(copies):
            for cp in copies:
                cp.start()

        def wait(copies):
            for cp in copies:
                cp.wait()

        def needs_next_weights(g, b):
            return jnp.logical_and(b == B - 1, g < NG - 1)

        def enqueue(t, may_be_past_end):
            g, b = group_batch(t)

            @pl.when(needs_next_weights(g, b))
            def _():
                start(w_copies(g + 1))

            if may_be_past_end:
                @pl.when(t < T)
                def _():
                    start(kv_copies(t))
            else:
                start(kv_copies(t))

        def project_q(t, j0, n):
            g, b = group_batch(t)
            cols = slice(j0 * Dh, (j0 + n) * Dh)
            q = jnp.dot(xb[b], wqb[g, :, cols], preferred_element_type=jnp.float32)
            qs[:, cols] = (q * q_scale).astype(qs.dtype)

        def step(t, last):
            g, b = group_batch(t)
            if last:
                start(out_copies(0, B - 1))
            else:
                @pl.when(needs_next_weights(g, b))
                def _():
                    wait(w_copies(g + 1))
            wait(kv_copies(t))

            h0 = g * HG
            scores, heads_out = {}, {}
            total = None
            for op, j in _parse(_LAST_STEP if last else _STEP):
                if op == "I":
                    enqueue(t + LA, True)
                elif op == "P":
                    project_q(t + 1, j, 1)
                elif op == "K":
                    scores[j] = jax.lax.dot_general(
                        qs[:, j * Dh:(j + 1) * Dh], kb[b, h0 + j], _NT,
                        preferred_element_type=jnp.float32)
                elif op == "V":
                    s = scores.pop(j)
                    m = jnp.max(s, axis=-1, keepdims=True)
                    p = jnp.exp2(s - m)
                    l = jnp.sum(p, axis=-1, keepdims=True)
                    o = jnp.dot(p.astype(vb.dtype), vb[b, h0 + j],
                                preferred_element_type=jnp.float32)
                    heads_out[j] = (o * pl.reciprocal(l, approx=False)).astype(wob.dtype)
                elif op == "O":
                    r = jnp.dot(heads_out.pop(j), wob[g, j * Dh:(j + 1) * Dh, :],
                                preferred_element_type=jnp.float32)
                    total = (acc[b] if total is None else total) + r
            if not last:
                acc[b] = total
            outb[b] = total.astype(outb.dtype)

        start(x_copies())
        start(w_copies(0))

        def fill(t, carry):
            enqueue(t, False)
            return carry

        jax.lax.fori_loop(0, LA, fill, 0)
        acc[...] = jnp.zeros(acc.shape, acc.dtype)
        wait(x_copies())
        wait(w_copies(0))
        project_q(0, 0, HG)

        def loop_step(t, carry):
            step(t, False)
            return carry

        jax.lax.fori_loop(0, T - 1, loop_step, 0)
        step(T - 1, True)

        start(out_copies(B - 1, 1))
        wait(out_copies(0, B - 1))
        wait(out_copies(B - 1, 1))

    hbm = pl.BlockSpec(memory_space=pl.ANY)
    return pl.pallas_call(
        kernel,
        in_specs=[hbm] * 5,
        out_specs=hbm,
        out_shape=jax.ShapeDtypeStruct((B, Sq, D), x.dtype),
        scratch_shapes=[
            pltpu.VMEM((B, Sq, D), x.dtype),
            pltpu.VMEM((B, H, Sk, Dh), k_cache.dtype),
            pltpu.VMEM((B, H, Sk, Dh), v_cache.dtype),
            pltpu.VMEM((NG, D, W), wq.dtype),
            pltpu.VMEM((NG, W, D), wo.dtype),
            pltpu.VMEM((B, Sq, D), jnp.float32),
            pltpu.VMEM((B, Sq, D), x.dtype),
            pltpu.VMEM((Sq, W), k_cache.dtype),
            pltpu.SemaphoreType.DMA((LA,)),
            pltpu.SemaphoreType.DMA((1,)),
        ],
        compiler_params=pltpu.CompilerParams(vmem_limit_bytes=100 * 2**20),
    )(x, k_cache, v_cache, wq, wo)
```
